```python
import os as _os
_os.environ.setdefault("JAX_PLATFORMS", "cpu")
import jax
import jax.numpy as jnp

def _softmax(x, axis=-1):
    return jax.nn.softmax(x, axis=axis)
def _gelu(x):
    return jax.nn.gelu(x, approximate=True)
def _silu(x):
    return jax.nn.silu(x)
def _sigmoid(x):
    return jax.nn.sigmoid(x)
def _layernorm(x, axis=-1, eps=1e-5):
    m = jnp.mean(x, axis=axis, keepdims=True)
    v = jnp.var(x, axis=axis, keepdims=True)
    return (x - m) / jnp.sqrt(v + eps)
def _scatter_add(tgt, idx, src, axis=0):
    return tgt.at[idx].add(src)
def _segment_sum(src, seg, n):
    return jax.ops.segment_sum(src, seg, n)
class _Rng:
    def __init__(self, key):
        self._k = key
    def _next(self):
        self._k, sub = jax.random.split(self._k)
        return sub
    def normal(self, shape):
        return jax.random.normal(self._next(), shape, dtype=jnp.bfloat16)
    def randint(self, lo, hi, shape):
        return jax.random.randint(self._next(), shape, lo, hi, dtype=jnp.int32)
    def uniform(self, shape, lo=0.0, hi=1.0):
        return jax.random.uniform(self._next(), shape, jnp.bfloat16, lo, hi)
    def permutation(self, n):
        return jax.random.permutation(self._next(), n)


kernel_name = 'gated_mix__linear_attn_block__sliding_local_dilated__prompt'

def setup_inputs():
    _rng = _Rng(jax.random.key(int.from_bytes(__import__("os").urandom(4), "little")))
    _w = (lambda a: (lambda t: t.astype(jnp.bfloat16) if jnp.issubdtype(t.dtype, jnp.floating) else t)(jnp.asarray(a)))
    def _A_setup():
        B, S, D = 1, 2048, 512
        return {
            "x": _w((lambda *s: _rng.normal(s) * 0.05)(B, S, D)),
            "wqkv": _w((lambda *s: _rng.normal(s) * 1.6)(D, 3 * D)),
            "wo": _w((lambda *s: _rng.normal(s) * 0.8)(D, D)),
        }
    _A_in = _A_setup()

    def _B_setup():
        B, S, D = 1, 2048, 512
        return {
            "x": _w((lambda *s: _rng.normal(s) * 0.05)(B, S, D)),
            "wqkv": _w((lambda *s: _rng.normal(s) * 0.8)(D, 3 * D)),
            "wo": _w((lambda *s: _rng.normal(s) * 0.05)(D, D)),
        }
    _B_in = _B_setup()

    return {
        "A_x": _A_in["x"],
        "A_wqkv": _A_in["wqkv"],
        "A_wo": _A_in["wo"],
        "B_x": _B_in["x"],
        "B_wqkv": _B_in["wqkv"],
        "B_wo": _B_in["wo"],
        "gate_w": _w((lambda *s: _rng.normal(s) * 0.05)(512) * 16.0),
    }

def reference(A_x, A_wqkv, A_wo, B_x, B_wqkv, B_wo, gate_w):
    def _A_ref(x, wqkv, wo):
        B, S, D = x.shape
        H = 32; Dh = D // H
        qkv = (lambda x, *d: x.transpose(*d))((x @ wqkv).reshape(B, S, 3, H, Dh), 2, 0, 3, 1, 4)
        q, k, v = qkv[0], qkv[1], qkv[2]
        phi = lambda t: jnp.where(t > 0, t + 1, jnp.exp(t)) + 1e-6
        pq, pk = phi(q), phi(k)
        kv = jnp.einsum("bhsd,bhse->bhde", pk, v)
        z = jnp.einsum("bhsd->bhd", pk)
        num = jnp.einsum("bhqd,bhde->bhqe", pq, kv)
        den = jnp.einsum("bhqd,bhd->bhq", pq, z)[..., None] + 1e-6
        o = num / den
        return (lambda x, *d: x.transpose(*d))(o, 0, 2, 1, 3).reshape(B, S, D) @ wo

    def _B_ref(x, wqkv, wo):
        B, S, D = x.shape
        H = 32; Dh = D // H
        W, dil = 8, 2
        qkv = (lambda x, *d: x.transpose(*d))((x @ wqkv).reshape(B, S, 3, H, Dh), 2, 0, 3, 1, 4)
        q, k, v = qkv[0], qkv[1], qkv[2]
        scale = Dh ** -0.5
        pos = jnp.arange(S)
        off = jnp.arange(W) * dil
        idx = pos[:, None] - off[None, :]
        mask = idx >= 0
        idx_c = jnp.where(mask, idx, 0).reshape(-1)
        kg = k[:, :, idx_c, :].reshape(B, H, S, W, Dh)
        vg = v[:, :, idx_c, :].reshape(B, H, S, W, Dh)
        logits = jnp.einsum("bhsd,bhswd->bhsw", q, kg) * scale
        logits = jnp.where(mask[None, None, :, :], logits, -1e9)
        attn = _softmax(logits, axis=-1)
        o = jnp.einsum("bhsw,bhswd->bhsd", attn, vg)
        return (lambda x, *d: x.transpose(*d))(o, 0, 2, 1, 3).reshape(B, S, D) @ wo

    x = A_x
    g = _sigmoid((x * gate_w).sum(-1, keepdims=True))
    a = _A_ref(x, A_wqkv, A_wo)
    b = _B_ref(x, B_wqkv, B_wo)
    return g * a + (1 - g) * b
```

```python
import functools
import jax
import jax.numpy as jnp
from jax import lax
import jax.experimental.pallas as pl
import jax.experimental.pallas.tpu as pltpu

S, D, H, DH, W, DIL = 2048, 512, 32, 16, 8, 2
PAD = 16
RB = 256
NB = S // RB
CH = 16
UNROLL = True
F32 = jnp.float32
BF16 = jnp.bfloat16


def _perm_tile(src_ref, jo):
    lane = lax.broadcasted_iota(jnp.int32, (D // 2, 128), 1)
    h = lane % 32
    idx = (h % 8) * 16 + 4 * jo + lane // 32
    acc = None
    for ji in range(4):
        u = pltpu.bitcast(src_ref[ji], jnp.uint32)
        g = jnp.take_along_axis(u, idx, axis=1)
        acc = g if acc is None else jnp.where(h // 8 == ji, g, acc)
    return pltpu.bitcast(acc, BF16)


def _phi(t):
    return jnp.where(t > 0, t + 1.0, jnp.exp(t)) + 1e-6


def _rcp(x):
    r = pl.reciprocal(x, approx=True)
    return r * (2.0 - x * r)


def _gsum(ts):
    u = (ts[0] + ts[1]) + (ts[2] + ts[3])
    u = u + pltpu.roll(u, 64, 1)
    u = u + pltpu.roll(u, 32, 1)
    return u


def _dot(a, b):
    return jnp.dot(a, b, preferred_element_type=F32)


def _kernel(x_hbm, aw_hbm, awo_hbm, bw_hbm, bwo_hbm, gw_ref, o_hbm,
            xs, wa, wb, wo, wap, wbp, wf, tmp, tmp2, pkT, q0, q1, k0, k1, v0, v1, oc0, oc1, ob0, ob1, ost, sems):
    def cp_w(src, c0, dst, t, sem):
        return pltpu.make_async_copy(src.at[:, pl.ds(c0 * 128, 128)], dst.at[t], sems.at[sem])
    def cp_x(i, j):
        return pltpu.make_async_copy(x_hbm.at[pl.ds(i * RB, RB), pl.ds(j * 128, 128)],
                                     xs.at[j, pl.ds(i * RB, RB), :], sems.at[i])
    SK, SQA, SVA, SWO, SB = NB, NB + 1, NB + 2, NB + 3, NB + 4
    wk_c = [cp_w(aw_hbm, 4 + t, wa, 4 + t, SK) for t in range(4)]
    x_c = [[cp_x(i, j) for j in range(4)] for i in range(NB)]
    wqa_c = [cp_w(aw_hbm, t, wa, t, SQA) for t in range(4)]
    wb_c = [[cp_w(bw_hbm, 4 * c + t, wb, 4 * c + t, SB + c) for t in range(4)] for c in range(3)]
    wva_c = [cp_w(aw_hbm, 8 + t, wa, 8 + t, SVA) for t in range(4)]
    wo_c = ([cp_w(awo_hbm, t, wo, t, SWO) for t in range(4)]
            + [cp_w(bwo_hbm, t, wo, 4 + t, SWO) for t in range(4)])
    def start(cs):
        for c in cs:
            c.start()
    start(wk_c + x_c[0]+x_c[1]+wqa_c)
    later = {0: x_c[2]+x_c[3]+wb_c[0], 1: x_c[4]+x_c[5]+wb_c[1], 3: x_c[6]+x_c[7]+wb_c[2], 4: wo_c+wva_c}

    def xblk(r0, n=RB):
        return jnp.concatenate([xs[j, pl.ds(r0, n), :] for j in range(4)], axis=1)

    def rowperm(tmp, dst_rows):
        for n in range(4):
            for d2 in range(8):
                t = jnp.concatenate([tmp[n, pl.ds(2 * d2 + e, 32, stride=16), :] for e in range(2)], axis=0)
                wf[n, pl.ds(dst_rows + d2 * 64, 64), :] = t.astype(BF16)

    for c in wk_c:
        c.wait()
    z = [jnp.zeros((8, 128), F32) for _ in range(4)]
    side = {1: (wqa_c, wa, 0, wap, 0), 3: (wb_c[0], wb, 0, wbp, 0), 5: (wb_c[1], wb, 4, wbp, 4), 7: (wb_c[2], wb, 8, wbp, 8)}
    row = lax.broadcasted_iota(jnp.int32, (128, 128), 0)
    col = lax.broadcasted_iota(jnp.int32, (128, 128), 1)
    for i in range(NB):
        for c in x_c[i]:
            c.wait()
        start(later.get(i, []))
        x = xblk(i * RB)
        for n in range(4):
            pk = _phi(_dot(x, wa[4 + n]))
            z[n] = z[n] + jnp.sum(pk.reshape(RB // 8, 8, 128), axis=0)
            pkT[pl.ds(n * 128, 128), pl.ds((i % 2) * RB, RB)] = pk.astype(BF16).T
        if i % 2 == 1:
            cs, src, s0, dst, d0 = side[i]
            for c in cs:
                c.wait()
            if i == NB - 1:
                for c in wo_c + wva_c:
                    c.wait()
            for b in range(4):
                Gs = []
                for n in range(4):
                    g = _dot(pkT[pl.ds(b * 128, 128), :], xs[n, pl.ds((i - 1) * RB, 2 * RB), :])
                    if i > 1:
                        g = g + tmp[n, pl.ds(b * 128, 128), :]
                    if i < NB - 1:
                        tmp[n, pl.ds(b * 128, 128), :] = g
                    Gs.append(g.astype(BF16))
                dst[d0 + b] = _perm_tile(src.at[pl.ds(s0, 4)], b)
                if i == NB - 1:
                    tmp2[b] = wo[4 + b].astype(F32)
                    kv = _dot(jnp.concatenate(Gs, axis=1), wa[8 + b])
                    kv = jnp.where(row // 16 == col // 16, kv, 0.0).astype(BF16)
                    for n in range(4):
                        tmp[n, pl.ds(b * 128, 128), :] = _dot(kv, wo[n, pl.ds(b * 128, 128), :])
    rowperm(tmp2, D)
    rowperm(tmp, 0)
    zs = [jnp.sum(z[n], axis=0, keepdims=True) for n in range(4)]
    lane = lax.broadcasted_iota(jnp.int32, (8, 128), 1)
    hh = lane % 32
    zp = []
    for jo in range(4):
        idx = (hh % 8) * 16 + 4 * jo + lane // 32
        acc = None
        for ji in range(4):
            g = jnp.take_along_axis(jnp.broadcast_to(zs[ji], (8, 128)), idx, axis=1)
            acc = g if acc is None else jnp.where(hh // 8 == ji, g, acc)
        zp.append(acc)
    zc = [jnp.concatenate([zp[j]] * (CH // 8), axis=0) for j in range(4)]
    gw = gw_ref[...].astype(F32).reshape(1, D)

    def att_chunk(i, c, slot):
        q2, k2, v2, oc2, ob_s = (q0, q1)[slot], (k0, k1)[slot], (v0, v1)[slot], (oc0, oc1)[slot], (ob0, ob1)[slot]
        r0 = i * RB
        rr = c * CH
        rows = pl.ds(rr, CH)
        xa = jnp.concatenate([xs[j, pl.ds(r0 + rr, CH), :] for j in range(4)], axis=1).astype(F32)
        g = _rcp(1.0 + jnp.exp(-jnp.sum(xa * gw, axis=1, keepdims=True)))
        pq = [oc2[j, rows, :] for j in range(4)]
        sc = g * _rcp(_gsum([pq[j] * zc[j] for j in range(4)]) + 1e-6)
        for j in range(4):
            ob_s[j, rows, :] = (pq[j] * sc).astype(BF16)
        q = [q2[j, rows, :] for j in range(4)]
        ls = []
        for w in range(W):
            l = _gsum([q[j] * k2[j, pl.ds(PAD + rr - DIL * w, CH), :] for j in range(4)])
            if i == 0 and rr < PAD and w:
                pos = rr + lax.broadcasted_iota(jnp.int32, (CH, 128), 0)
                l = jnp.where(pos >= DIL * w, l, -1e9)
            ls.append(l)
        m = functools.reduce(jnp.maximum, ls)
        es = [jnp.exp(l - m) for l in ls]
        inv = (1.0 - g) * _rcp(functools.reduce(lambda a, b: a + b, es))
        for j in range(4):
            acc = None
            for w in range(W):
                t = es[w] * v2[j, pl.ds(PAD + rr - DIL * w, CH), :]
                acc = t if acc is None else acc + t
            ob_s[4 + j, rows, :] = (acc * inv).astype(BF16)

    pass

    def proj(i, p):
        slot = i % 2
        q2, k2, v2, oc2 = (q0, q1)[slot], (k0, k1)[slot], (v0, v1)[slot], (oc0, oc1)[slot]
        x = xblk(i * RB)
        if p < 4:
            oc2[p] = _phi(_dot(x, wap[p]))
        elif p < 8:
            q2[p - 4] = _dot(x, wbp[p - 4]) * (DH ** -0.5)
        else:
            ref = k2 if p < 12 else v2
            prev = ((k0, k1) if p < 12 else (v0, v1))[1 - slot]
            n = p % 4
            ref[n, pl.ds(PAD, RB), :] = _dot(x, wbp[p - 4])
            if i == 0:
                ref[n, 0:PAD, :] = jnp.zeros((PAD, 128), F32)
            else:
                ref[n, 0:PAD, :] = prev[n, pl.ds(RB, PAD), :]

    out_c = {}
    def final(i, n):
        slot = i % 2
        ob_s = (ob0, ob1)[slot]
        lhs = jnp.concatenate([ob_s[j] for j in range(8)], axis=1)
        ost[n, pl.ds(i * RB, RB), :] = _dot(lhs, wf[n]).astype(BF16)
    def out_cp(i, n):
        return pltpu.make_async_copy(ost.at[n, pl.ds(i * RB, RB), :], o_hbm.at[pl.ds(i * RB, RB), pl.ds(n * 128, 128)], sems.at[SB + 3])

    NC = RB // CH
    for p in range(16):
        proj(0, p)
    for i in range(NB + 1):
        pieces = []
        if i + 1 < NB:
            pieces += [functools.partial(proj, i + 1, p) for p in range(16)]
        if i >= 1:
            fin = [functools.partial(final, i - 1, n) for n in range(4)]
            pieces = fin + pieces
        chunks = [functools.partial(att_chunk, i, c, i % 2) for c in range(NC)] if i < NB else []
        wts = ([2] * 4 if i >= 1 else []) + ([1] * 16 if i + 1 < NB else [])
        tot, nc = sum(wts), len(chunks)
        ci = 0
        acc = 0
        for wt, pc in zip(wts, pieces):
            pc()
            acc += wt
            while ci < nc and ci * tot < acc * nc:
                chunks[ci]()
                ci += 1
        if i >= 1:
            for n in range(4):
                out_cp(i - 1, n).start()
    for i in range(NB):
        for n in range(4):
            out_cp(i, n).wait()


@jax.jit
def pallas_gated_mix__linear_attn_block__sliding_local_dilated__prompt_kernel(
    A_x, A_wqkv, A_wo, B_x, B_wqkv, B_wo, gate_w):
    anyspec = pl.BlockSpec(memory_space=pl.ANY)
    out = pl.pallas_call(
        _kernel,
        out_shape=jax.ShapeDtypeStruct((S, D), BF16),
        in_specs=[anyspec] * 5 + [pl.BlockSpec(memory_space=pltpu.VMEM)],
        out_specs=anyspec,
        scratch_shapes=[
            pltpu.VMEM((4, S, 128), BF16),
            pltpu.VMEM((12, D, 128), BF16),
            pltpu.VMEM((12, D, 128), BF16),
            pltpu.VMEM((8, D, 128), BF16),
            pltpu.VMEM((4, D, 128), BF16),
            pltpu.VMEM((12, D, 128), BF16),
            pltpu.VMEM((4, 2 * D, 128), BF16),
            pltpu.VMEM((4, D, 128), F32),
            pltpu.VMEM((4, D, 128), F32),
            pltpu.VMEM((D, 2 * RB), BF16),
            *[pltpu.VMEM((4, RB, 128), F32)] * 2,
            *[pltpu.VMEM((4, RB + PAD, 128), F32)] * 4,
            *[pltpu.VMEM((4, RB, 128), F32)] * 2,
            *[pltpu.VMEM((8, RB, 128), BF16)] * 2,
            pltpu.VMEM((4, S, 128), BF16),
            pltpu.SemaphoreType.DMA((NB + 10,)),
        ],
        compiler_params=pltpu.CompilerParams(vmem_limit_bytes=100 * 1024 * 1024),
    )(A_x.reshape(S, D), A_wqkv, A_wo, B_wqkv, B_wo, gate_w)
    return out.reshape(1, S, D)
```
